```python
import os as _os
_os.environ.setdefault("JAX_PLATFORMS", "cpu")
import jax
import jax.numpy as jnp

def _softmax(x, axis=-1):
    return jax.nn.softmax(x, axis=axis)
def _gelu(x):
    return jax.nn.gelu(x, approximate=True)
def _silu(x):
    return jax.nn.silu(x)
def _sigmoid(x):
    return jax.nn.sigmoid(x)
def _layernorm(x, axis=-1, eps=1e-5):
    m = jnp.mean(x, axis=axis, keepdims=True)
    v = jnp.var(x, axis=axis, keepdims=True)
    return (x - m) / jnp.sqrt(v + eps)
def _scatter_add(tgt, idx, src, axis=0):
    return tgt.at[idx].add(src)
def _segment_sum(src, seg, n):
    return jax.ops.segment_sum(src, seg, n)
class _Rng:
    def __init__(self, key):
        self._k = key
    def _next(self):
        self._k, sub = jax.random.split(self._k)
        return sub
    def normal(self, shape):
        return jax.random.normal(self._next(), shape, dtype=jnp.bfloat16)
    def randint(self, lo, hi, shape):
        return jax.random.randint(self._next(), shape, lo, hi, dtype=jnp.int32)
    def uniform(self, shape, lo=0.0, hi=1.0):
        return jax.random.uniform(self._next(), shape, jnp.bfloat16, lo, hi)
    def permutation(self, n):
        return jax.random.permutation(self._next(), n)


kernel_name = 'standalone__mixer_token_mlp__sampling'

def setup_inputs():
    _rng = _Rng(jax.random.key(int.from_bytes(__import__("os").urandom(4), "little")))
    _w = (lambda a: (lambda t: t.astype(jnp.bfloat16) if jnp.issubdtype(t.dtype, jnp.floating) else t)(jnp.asarray(a)))
    B, S, D, F = 32, 16, 1024, 3584
    return {
        "x": _w((lambda *s: _rng.normal(s) * 0.05)(B, S, D)),
        "w1": _w((lambda *s: _rng.normal(s) * 0.05)(S, F) * (S ** -0.5)),
        "b1": _w((lambda *s: _rng.normal(s) * 0.05)(F) * 0.02),
        "w2": _w((lambda *s: _rng.normal(s) * 0.05)(F, S) * (F ** -0.5)),
        "b2": _w((lambda *s: _rng.normal(s) * 0.05)(S) * 0.02),
    }

def reference(x, w1, b1, w2, b2):
    B, S, D = x.shape
    h = _layernorm(x, axis=-1)
    u = jnp.einsum("bsd,sf->bdf", h, w1) + b1
    u = _gelu(u)
    y = jnp.einsum("bdf,fs->bds", u, w2) + b2
    return (lambda x, *d: x.transpose(*d))(y, 0, 2, 1)
```

```python
import functools, numpy as np, jax, jax.numpy as jnp
from jax import lax
import jax.experimental.pallas as pl
import jax.experimental.pallas.tpu as pltpu

C1 = float(np.sqrt(2 / np.pi)); C2 = C1 * 0.044715
A = float(np.cbrt(C2)); K = C1 / A
bf16 = jnp.bfloat16; f32 = jnp.float32
A_HI = float(np.float32(A).astype(bf16)); A_LO = A - A_HI
NT = 512; NL = NT // 128

def make(R=(1, 2), R0=(), R1=(), lead=17, NB=1, vpos=8, lnpos=3, hpos=8, flags=None, chain=0, accmem=0, rawc=0, lead1=None, nacc=1, lnseq=0, SS=8, HP=8, bpos=1, bar='sum', hstep=0, oz=0):
    B, S, D, F = 32, 16, 1024, 3584
    NC = F // 128; NH = D // NT; U = NB * NH; KA = 24; ND = D // 128
    tiles = []
    for q in range(U):
        for j in range(NC):
            t = q * NC + j
            r = R0[t] if t < len(R0) else R1[t - U * NC] if t >= U * NC - len(R1) else R[j % len(R)]
            c = NC - 1 - j
            gs = [c * 16 + k for k in range(15, -1, -1)]
            if not isinstance(r, tuple): r = tuple(range(min(vpos, 16 - r), min(vpos, 16 - r) + r))
            tiles.append((q, j, c, gs, [gs[p] for p in r]))
    vp = sorted({g for t in tiles for g in t[4]})
    mx = []; ends = []
    for q, j, c, gs, vs in tiles:
        if j == 0: mx += [(q, 'L1'), (q, 'L0')]
        mx += [(q, g) for g in gs if g not in vs]
        ends.append(len(mx))
    L = len(mx); ncarry = lead if lead1 is None else lead1
    HF = 16 * ND

    hrow = lambda s, i: (i * 16 + s) * SS + i * HP
    HE = hrow(0, ND)
    def kern(x_hbm, w1_hbm, b1_hbm, w2t_hbm, b2_hbm, o_hbm, x_v, w1_v, b1_v, w2t_v, b2_v, o_v, w1t_s, w2_s, wbc_s, hk_s, h_s, hf_s, carry_s, sems, osem):
        lanes = lambda vs: jnp.concatenate(list(vs), axis=1)
        rows = lambda vs: jnp.concatenate(list(vs), axis=0)
        cps = [pltpu.make_async_copy(s, d, sems.at[i]) for i, (s, d) in enumerate([
            (w1_hbm, w1_v), (b1_hbm, b1_v), (x_hbm.at[pl.ds(0, NB)], x_v.at[pl.ds(0, NB)]), (w2t_hbm, w2t_v), (b2_hbm, b2_v),
            (x_hbm.at[pl.ds(NB, B - NB)], x_v.at[pl.ds(NB, B - NB)])])]
        for cp in cps: cp.start()
        for cp in cps[:5]: cp.wait()

        def layernorm(b, slot):
            x = x_v[b].astype(f32)
            m = jnp.mean(x, axis=-1, keepdims=True)
            xc = x - m
            v = jnp.mean(xc * xc, axis=-1, keepdims=True)
            h = (xc * (A * lax.rsqrt(v + 1e-5))).astype(bf16).astype(f32)
            for i in range(ND):
                hf_s[slot, :, i * 128:(i + 1) * 128] = h[:, i * 128:(i + 1) * 128]
        def stage(slot, n, pieces=range(2 * NL), z=0):
            for p in pieces:
                i, r = n * NL + p // 2, p % 2
                h = hf_s[slot, r * 8:(r + 1) * 8, i * 128:(i + 1) * 128]
                hk_s[r * 8:(r + 1) * 8, i * 128:(i + 1) * 128] = h
                for k in range(8): h_s[pl.ds(hrow(r * 8, i) + k, 8, stride=SS), :] = h

        ri = lax.broadcasted_iota(jnp.int32, (8, 128), 0)
        hk_s[16:KA, :] = lanes([jnp.where(ri == 0, A_HI, jnp.where(ri == 1, A_LO, 0.0))] * ND)
        for k in range(NB): layernorm(k, k)
        stage(0, 0)
        b1 = b1_v[...].astype(f32)
        wc = jnp.zeros((16, 128), f32)
        for c in range(NC - 1, -1, -1):
            bt = jnp.where(ri < 2, jnp.broadcast_to(b1[c:c + 1, :], (8, 128)), 0.0)
            wa = rows([w1_v[:, c * 128:(c + 1) * 128].astype(f32), bt, jnp.zeros((104, 128), f32)])
            wt = wa.T
            w1t_s[c * 128:(c + 1) * 128, :] = wt
            w2c = w2t_v[:, c * 128:(c + 1) * 128].astype(f32)
            w2_s[:, c * 128:(c + 1) * 128] = w2c
            wc = wc + jnp.dot(w2c, wt, preferred_element_type=f32)
            for g in vp:
                if g // 16 == c:
                    row = wt[(g % 16) * 8:(g % 16 + 1) * 8]
                    for s in range(17):
                        col = row[:, s:s + 1]
                        wbc_s[vp.index(g), s] = jnp.broadcast_to(col * A if s == 16 else col, (8, 128))
        l16 = lax.broadcasted_iota(jnp.int32, (16, 128), 1)
        e16 = lax.broadcasted_iota(jnp.int32, (16, 16), 0) == lax.broadcasted_iota(jnp.int32, (16, 16), 1)
        b2c = jnp.sum(jnp.where(e16, jnp.broadcast_to(b2_v[...].astype(f32), (16, 16)), 0.0), axis=1, keepdims=True)
        wc = wc + jnp.where((l16 == 16) | (l16 == 17), 2.0 * b2c, 0.0)
        wc_hi = wc.astype(bf16).astype(f32)
        w1t_s[F:F + 16, :] = wc_hi + pltpu.roll(wc - wc_hi, KA, 1)

        def act(u):
            return u * jnp.tanh(u * (u * u + K))

        def mm1(items, us):
            n = items[0][0] % NH
            hh = hk_s[:, n * NT:(n + 1) * NT]
            kk = KA
            if any(isinstance(g, str) for _, g in items):
                hh = rows([hh, hh]); kk = 2 * KA
            gi = [F // 8 + int(g[1]) if isinstance(g, str) else g for _, g in items]
            u = jnp.dot(rows(w1t_s[g * 8:(g + 1) * 8, :kk] for g in gi), hh, preferred_element_type=f32)
            for i, key in enumerate(items): us[key] = u[i * 8:(i + 1) * 8]

        cooked = set(mx[:ncarry - rawc])
        def put_carry(us):
            for i, key in enumerate(mx[:ncarry]):
                carry_s[i] = act(us[key]) if key in cooked and not isinstance(key[1], str) else us[key]
        us0 = {}
        mm1(mx[:ncarry], us0); put_carry(us0)
        cps[5].wait()
        out_cp = lambda it: pltpu.make_async_copy(o_v.at[pl.ds(it * NB, NB)], o_hbm.at[pl.ds(it * NB, NB)], osem)

        def body(it, cur):
            us = {key: carry_s[i] for i, key in enumerate(mx[:ncarry])}; nxt = {}; acc = None
            oth = NB - cur; z = cur * oth if oz else 0
            pos = ncarry
            rep = lambda v: lanes([v] * NL)
            for t, (q, j, c, gs, vs) in enumerate(tiles):
                k, n = divmod(q, NH)
                if t == bpos:
                    v = hk_s[16:24, 0:128]
                    v = jnp.broadcast_to(jnp.sum(v, axis=1, keepdims=True), (8, 128)) if bar == 'sum' else pltpu.roll(v, 1, 1)
                    h_s[pl.ds(pl.multiple_of(-(-HE // 8) * 8 + cur * 8, 8), 8), :] = v
                if j == lnpos and n == lnseq: layernorm(jnp.minimum((it + 1) * NB + k, B - 1), oth + k)
                stage(oth if q == U - 1 else cur + (q + 1) // NH, (n + 1) % NH, [p for p in range(2 * NL) if hpos + p * hstep == j], z)
                end = ends[t] + (lead if t < len(tiles) - 1 else ncarry)
                while pos < end:
                    p = pos % L; e = p
                    while e < L and e - p < end - pos and mx[e][0] == mx[p][0]: e += 1
                    mm1(mx[p:e], us if pos < L else nxt)
                    pos += e - p
                for g in vs:
                    parts = [rep(wbc_s[vp.index(g), 16])] + [None] * (nacc - 1)
                    for s in range(16):
                        pr = rep(wbc_s[vp.index(g), s]) * lanes(h_s[hrow(s, i):hrow(s, i) + 8, :] for i in range(n * NL, (n + 1) * NL))
                        parts[s % nacc] = pr if parts[s % nacc] is None else parts[s % nacc] + pr
                    us[q, g] = functools.reduce(lambda a, b: a + b, parts)
                if j == 0:
                    lin = rows([us.pop((q, 'L0')), us.pop((q, 'L1'))])
                    acc = jnp.where(it < 0, acc, lin) if chain and q else lin
                gl = {g: us.pop((q, g)) if (q, g) in cooked else act(us.pop((q, g))) for g in gs}
                if t == len(tiles) - 1: put_carry(nxt)
                acc = acc + jnp.dot(w2_s[:, c * 128:(c + 1) * 128], rows(gl[i] for i in sorted(gs)), preferred_element_type=f32)
                if j == NC - 1: fin = acc
                if accmem and j == accmem and q:
                    for i in range(2):
                        for l in range(NL): h_s[HF + 2 * NB * 2 * ND + z + i * NL + l] = fin[i * 8:(i + 1) * 8, l * 128:(l + 1) * 128]
                if j == NC - 1:
                    o_v[it * NB + k, :, n * NT:(n + 1) * NT] = ((0.5 / A) * acc).astype(bf16)
            out_cp(it).start()
            return oth
        lax.fori_loop(0, B // NB, body, 0)
        pltpu.make_async_copy(o_v, o_hbm, osem).wait()

    def fn(x, w1, b1, w2, b2):
        hbm = pl.BlockSpec(memory_space=pltpu.HBM)
        return pl.pallas_call(kern,
            in_specs=[hbm] * 5, out_specs=hbm,
            out_shape=jax.ShapeDtypeStruct(x.shape, x.dtype),
            scratch_shapes=[pltpu.VMEM((B, S, D), bf16), pltpu.VMEM((S, F), bf16), pltpu.VMEM((NC, 128), bf16), pltpu.VMEM((S, F), bf16),
                            pltpu.VMEM((1, S), bf16), pltpu.VMEM((B, S, D), bf16),
                            pltpu.VMEM((F + 16, 128), f32), pltpu.VMEM((S, F), f32), pltpu.VMEM((len(vp), 17, 8, 128), f32),
                            pltpu.VMEM((KA, D), f32), pltpu.VMEM((HE + 8 * (NB + 1), 128), f32), pltpu.VMEM((2 * NB, S, D), f32), pltpu.VMEM((ncarry, 8, NT), f32),
                            pltpu.SemaphoreType.DMA((6,)), pltpu.SemaphoreType.DMA(())],
            compiler_params=pltpu.CompilerParams(vmem_limit_bytes=64 * 2**20, flags=flags),
        )(x, w1, b1.reshape(NC, 128), w2.T, b2.reshape(1, S))
    return fn


_fn = make(lnseq=1, R0=((1, 6, 11), 1), SS=9, HP=0)

@jax.jit
def pallas_standalone__mixer_token_mlp__sampling_kernel(x, w1, b1, w2, b2):
    return _fn(x, w1, b1, w2, b2)
```

```python
import functools, numpy as np, jax, jax.numpy as jnp
from jax import lax
import jax.experimental.pallas as pl
import jax.experimental.pallas.tpu as pltpu
C1 = float(np.sqrt(2 / np.pi)); C2 = C1 * 0.044715
A = float(np.cbrt(C2)); K = C1 / A
bf16 = jnp.bfloat16; f32 = jnp.float32
A_HI = float(np.float32(A).astype(bf16)); A_LO = A - A_HI

def quads(m):
    n = len(m) // 2
    return [[row[j * n:(j + 1) * n] for row in m[i * n:(i + 1) * n]] for i in range(2) for j in range(2)]
def zipm(f, a, b): return [[f(x, y) for x, y in zip(r, s)] for r, s in zip(a, b)]
madd = functools.partial(zipm, lambda x, y: x + y)
msub = functools.partial(zipm, lambda x, y: x - y)
def sw_left(a):
    if len(a) == 1: return [a[0][0]]
    a11, a12, a21, a22 = quads(a)
    s1 = madd(a21, a22); s2 = msub(s1, a11); s3 = msub(a11, a21); s4 = msub(a12, s2)
    return [v for m in (a11, a12, s4, a22, s1, s2, s3) for v in sw_left(m)]
def sw_right(b):
    if len(b) == 1: return [b[0][0]]
    b11, b12, b21, b22 = quads(b)
    t1 = msub(b12, b11); t2 = msub(b22, t1); t3 = msub(b22, b12); t4 = msub(t2, b21)
    return [v for m in (b11, b21, b22, t4, t1, t2, t3) for v in sw_right(m)]
def sw_bias(b):
    if len(b) == 1: return {0: b[0]}
    n = len(b) // 2; k = 7 ** (n.bit_length() - 1)
    out = dict(sw_bias(b[:n]))
    out.update({6 * k + i: v for i, v in sw_bias([y - x for x, y in zip(b[:n], b[n:])]).items()})
    return out
def sw_out(p):
    if len(p) == 1: return [[p[0]]]
    k = len(p) // 7
    p1, p2, p3, p4, p5, p6, p7 = (sw_out(p[i * k:(i + 1) * k]) for i in range(7))
    u2 = madd(p1, p6); u3 = madd(u2, p7)
    c11 = madd(p1, p2); c12 = madd(madd(u2, p5), p3); c21 = msub(u3, p4); c22 = madd(u3, p5)
    return [r + s for r, s in zip(c11, c12)] + [r + s for r, s in zip(c21, c22)]

bf16 = jnp.bfloat16; f32 = jnp.float32; i32 = jnp.int32
NT = 512; NL = NT // 128; KA = 32

def make(U=7, LV=1, NV=46, lo=6, hi=222, gap=None, X=(), vp=None, lead=18, hpos=10, bpos=1, Lpos=0, Lp0=20, SS=9, flags=None, lead0=16,
         nln=3, alag=2, aper=4, skip={0: (2,)}, npre=4, dstart=True, swap=False, raw=2, leads={}, dbc=True, trips=None, pret=False, npc=7, hstep=2, hbar=True, l0=3, l1=26, pre=0):
    B, S, D, F = 32, 16, 1024, 3584
    NC = F // 128; NH = D // NT; NG = F // 8; NS = B * NH
    M = 2 ** LV; NP = 7 ** LV; KS = S // M; CW = NL // M
    order = list(range(NG - 1, -1, -1))
    npr = NV // 2
    if vp is None:
        if gap is None: vp = [int(round(lo + i * (hi - lo) / (npr - 1))) for i in range(npr)]
        else: vp = [int(round(lo + u * (hi - lo - gap) / (npr // 2 - 1))) + k * gap for u in range(npr // 2) for k in range(2)]
    assert not set(X) & set(vp)
    gsl = [order[2 * p + k] for p in list(vp) + list(X) for k in range(2)]
    allu = [gsl[i:i + M] for i in range(0, len(gsl), M)]
    nu = 2 * len(vp) // M
    uns_of = lambda q: [i for i in range(len(allu) if q == 0 else nu) if i not in skip.get(q, ())]
    NIT = (NS - 1) // U
    assert 1 + NIT * U == NS
    hrow = lambda p, s, l: (((p * KS + s) // 8 * CW + l) * 8 + (p * KS + s) % 8) * SS
    NTV = -(-NP * KS // 8) * CW
    HE = NTV * 8 * SS

    B0 = max(min((1 + (i + 1) * U) // NH, B - 1) + 1 - i * nln for i in range(NIT))
    def stream(q, uns, lp):
        v = {g for i in uns for g in allu[i]}
        out = []; ends = []
        for j in range(NC):
            if j == lp: out += [(q, NG + 1), (q, NG)]
            out += [(q, g) for g in order[j * 16:(j + 1) * 16] if g not in v]
            ends.append(len(out))
        return out, ends
    head = stream(0, uns_of(0), Lpos)[0][:lead]

    def kern(x_hbm, w1_hbm, b1_hbm, w2t_hbm, b2_hbm, o_hbm, x_v, w1_v, b1_v, w2t_v, b2_v, o_v, w1t_s, w2_s, wbc_s, hk_s, h_s, hn_s, ht_s, carry_s, sems, osem):
        lanes = lambda vs: jnp.concatenate(list(vs), axis=1)
        rows = lambda vs: jnp.concatenate(list(vs), axis=0)
        pk = lambda v: pltpu.bitcast(v.astype(bf16), i32)
        unpk = lambda v: pltpu.bitcast(v, bf16)
        cps = [pltpu.make_async_copy(s, d, sems.at[i]) for i, (s, d) in enumerate([
            (x_hbm.at[pl.ds(0, B0)], x_v.at[pl.ds(0, B0)]), (w1_hbm, w1_v), (b1_hbm, b1_v), (w2t_hbm, w2t_v), (b2_hbm, b2_v),
            (x_hbm.at[pl.ds(B0, B - B0)], x_v.at[pl.ds(B0, B - B0)])])]
        for cp in cps[:5]: cp.start()

        def combos(hp):
            h = unpk(hp).astype(f32)
            if KS >= 8:
                ts = sw_right([[h[k * KS:(k + 1) * KS, j * CW * 128:(j + 1) * CW * 128] for j in range(M)] for k in range(M)])
                return [t[r:r + 8, l * 128:(l + 1) * 128] for t in ts for r in range(0, KS, 8) for l in range(CW)]
            hr = rows([pltpu.roll(h[:8], 4, 0), pltpu.roll(h[8:], 4, 0)])
            ts = sw_right([[(hr if k % 2 else h)[k // 2 * 8:k // 2 * 8 + 8, j * 128:(j + 1) * 128] for j in range(M)] for k in range(M)])
            low = lax.broadcasted_iota(i32, (8, 128), 0) < 4
            return [jnp.where(low, ts[i], pltpu.roll(ts[min(i + 1, NP - 1)], 4, 0)) for i in range(0, NP, 2)]
        def layernorm(b0, nb):
            x = x_v[pl.ds(b0, nb)].reshape(nb * S, D).astype(f32)
            m = jnp.mean(x, axis=-1, keepdims=True)
            xc = x - m
            v = jnp.mean(xc * xc, axis=-1, keepdims=True)
            h = pk(xc * (A * lax.rsqrt(v + 1e-5)))
            for b in range(nb):
                for n in range(NH):
                    hn_s[(b0 + b) * NH + n] = h[b * 8:(b + 1) * 8, n * NT:(n + 1) * NT]
                    if pret:
                        for i, t in enumerate(combos(h[b * 8:(b + 1) * 8, n * NT:(n + 1) * NT])): ht_s[(b0 + b) * NH + n, i] = t
            return h
        def stage(seq, buf, vpu=True, piece=None):
            hp = hk_s[buf, 0:8, :] if piece else hn_s[seq]
            if not piece: hk_s[buf, 0:8, :] = hp
            if not vpu: return
            ts = [ht_s[seq, i] for i in range(NTV)] if pret else combos(hp)
            for i, t in enumerate(ts):
                if piece is not None and i * npc // NTV != piece: continue
                for k in range(8): h_s[buf][pl.ds(i * 8 * SS + k, 8, stride=SS), :] = t

        def act(u):
            return u * jnp.tanh(u * (u * u + K))

        def mm1(items, buf, us, ones=None):
            hh = unpk(hk_s[buf] if ones is None else rows([hk_s[buf, 0:8, :], lanes([ones] * NL)])); kk = KA
            if any(g >= NG for _, g in items):
                hh = rows([hh, hh]); kk = 2 * KA
            u = jnp.dot(unpk(rows(w1t_s[g // 2] for _, g in items[1::2]))[:, :kk], hh, preferred_element_type=f32)
            for i, key in enumerate(items):
                if not swap or key[1] >= NG: i ^= 1
                us[key] = u[i * 8:(i + 1) * 8]

        def vpu(iu, buf):
            rep = lambda v: lanes([v] * CW)
            bias = {p: i for i, p in enumerate(sw_bias([0] * M))}
            ps = []
            for p in range(NP):
                acc = rep(wbc_s[iu, NP * KS + bias[p]]) if p in bias else None
                for s in range(KS):
                    pr = rep(wbc_s[iu, p * KS + s]) * lanes(h_s[buf][hrow(p, s, l):hrow(p, s, l) + 8, :] for l in range(CW))
                    acc = pr if acc is None else acc + pr
                ps.append(acc)
            return [lanes(r) for r in sw_out(ps)]

        def put(sq):
            pltpu.make_async_copy(o_v.at[sq], o_hbm.at[sq // NH, :, pl.ds(pl.multiple_of(sq % NH * NT, NT), NT)], osem).start()

        def block(seq0, specs, ld, carried, side, z=None):
            mx = []; ends = []
            for q, (buf, uns, lp) in enumerate(specs):
                st, en = stream(q, uns, lp)
                ends += [len(mx) + e for e in en]; mx += st
            last = len(specs)
            mx += [(last, g) for _, g in head]
            us = {key: carry_s[i] for i, key in enumerate(head)} if carried else {}
            pos = len(us); done = set(head[:lead - raw]) if carried else (); accs = {}
            for t in range(len(ends)):
                q, j = divmod(t, NC)
                buf, uns, lp = specs[q]
                ones = side(q, j)
                end = min(ends[t] + (leads.get(t, ld) if carried else ld), len(mx)) if t < len(ends) - 1 else len(mx) - raw
                while pos < end:
                    e = pos
                    while e < end and mx[e][0] == mx[pos][0]: e += 1
                    mm1(mx[pos:e], specs[mx[pos][0]][0] if mx[pos][0] < last else 0, us, ones)
                    pos = e
                gs = order[j * 16:(j + 1) * 16]
                for i in uns:
                    if allu[i][0] in gs:
                        for g, v in zip(allu[i], vpu(i, buf)): us[q, g] = v
                gl = {g: us.pop((q, g)) if (q, g) in done else act(us.pop((q, g))) for g in gs}
                c = NC - j
                if z is not None and t - alag in accs:
                    w2_s[0] = accs.pop(t - alag); c = c + z * (1 - z)
                y = lax.dot_general(unpk(w2_s[c, :8, :128]), rows(gl[g] for g in sorted(gs)), (((1,), (0,)), ((), ())), preferred_element_type=f32)
                acc = y if j == 0 else acc + y
                if j == lp: acc = acc + rows([us.pop((q, NG)), us.pop((q, NG + 1))])
                if aper and j % aper == aper - 1: accs[t] = acc
                if j == NC - 1: o_v[seq0 + q] = ((0.5 / A) * acc).astype(bf16)
            if raw: mm1(mx[pos:], 0, us)
            for i, (_, g) in enumerate(head): carry_s[i] = us[last, g] if g >= NG or i >= lead - raw else act(us[last, g])

        ri = lax.broadcasted_iota(i32, (16, 128), 0)
        for buf in range(U + 1): hk_s[buf, 8:16, :] = lanes([pk(jnp.where(ri == 0, A_HI, jnp.where(ri == 1, A_LO, 0.0)))] * NL)
        for buf in range(U): h_s[buf][HE + 16:HE + 32, :] = rows([pltpu.bitcast(hk_s[0, 8:16, :128], f32)] * 2)
        cps[0].wait()
        layernorm(0, B0); stage(0, U, False)
        cps[1].wait(); cps[2].wait()
        b1 = b1_v[...].astype(f32)
        was = {}
        for c in range(NC - 1, -1, -1):
            if c == NC - 1 - npre: cps[3].wait(); cps[4].wait(); cps[5].start()
            bt = jnp.where(ri < 2, jnp.broadcast_to(b1[c:c + 1, :], (16, 128)), 0.0).astype(bf16)
            was[c] = rows([w1_v[:, c * 128:(c + 1) * 128], bt])
            wt = rows([was[c], jnp.zeros((96, 128), bf16)]).T
            if swap:
                wt = wt.astype(f32)
                wt = rows(wt[(i ^ 1) * 8:((i ^ 1) + 1) * 8] for i in range(16))
            w1t_s[c * 8:(c + 1) * 8] = pk(wt).reshape(8, 8, 128)
        for c in range(NC): w2_s[c + 1, :8, :128] = pltpu.bitcast(w2t_v[:, c * 128:(c + 1) * 128], f32)
        def linear():
            wa = lanes(was[c] for c in range(NC))
            wc = lax.dot_general(w2t_v[...], wa, (((1,), (1,)), ((), ())), preferred_element_type=f32)
            wc = lanes([wc, jnp.zeros((16, 128 - KA), f32)])
            l16 = lax.broadcasted_iota(i32, (16, 128), 1)
            e16 = lax.broadcasted_iota(i32, (16, 16), 0) == lax.broadcasted_iota(i32, (16, 16), 1)
            b2c = jnp.sum(jnp.where(e16, jnp.broadcast_to(b2_v[...].astype(f32), (16, 16)), 0.0), axis=1, keepdims=True)
            wc = wc + jnp.where((l16 == 16) | (l16 == 17), 2.0 * b2c, 0.0)
            wc_hi = wc.astype(bf16).astype(f32)
            w1t_s[NG // 2] = pk(wc_hi + pltpu.roll(wc - wc_hi, KA, 1))
        def tables():
            def bc(g, s):
                v = unpk(jnp.broadcast_to(w1t_s[g // 2][:, s:s + 1], (8, 128))).astype(f32)
                i = (g % 2) ^ int(swap)
                return v[i * 8:(i + 1) * 8]
            for iu, un in enumerate(allu):
                for i, v in enumerate(sw_bias([A * bc(g, 16) for g in un]).values()): wbc_s[iu, NP * KS + i] = v
            for s in range(KS):
                for iu, un in enumerate(allu):
                    for p, v in enumerate(sw_left([[bc(g, k * KS + s) for k in range(M)] for g in un])): wbc_s[iu, p * KS + s] = v
        def side0(q, j):
            if j == pre: linear()
            if j == 0: tables(); stage(1, 0)
        block(0, [(U, [], Lp0)], lead0, False, side0)
        put(0)
        cps[5].wait()

        def body(it, z):
            seq0 = 1 + it * U
            v = pltpu.roll(wbc_s[0, 0], 1, 1)
            def side(q, j):
                if j == (bpos if q == 0 else 0): h_s[q][pl.ds(pl.multiple_of(HE + z * 8, 8), 8), :] = v
                if j >= hpos and (j - hpos) % hstep == 0 and (j - hpos) // hstep < npc:
                    stage(jnp.minimum(seq0 + q + 1, NS - 1), (q + 1) % U, True, (j - hpos) // hstep)
                    if hbar: return pltpu.bitcast(h_s[(q + 1) % U][pl.ds(pl.multiple_of(HE + 16 + z * 8, 8), 8), :], i32)
                if dstart and q and j == 3: put(seq0 + q - 1)
            block(seq0, [(q, uns_of(q), Lpos) for q in range(U)], lead, True, side, z)
            for q in range(U - 1 if dstart else 0, U): put(seq0 + q)
            layernorm(jnp.minimum(B0 + it * nln, B - nln), nln)
            return 1 - z
        nit = NIT if trips is None else trips
        if nit: lax.fori_loop(0, nit, body, 0)
        pltpu.make_async_copy(o_v.at[pl.ds(0, 1 + nit * U)], o_v.at[pl.ds(0, 1 + nit * U)], osem).wait()

    def fn(x, w1, b1, w2, b2):
        hbm = pl.BlockSpec(memory_space=pltpu.HBM)
        return pl.pallas_call(kern,
            in_specs=[hbm] * 5, out_specs=hbm,
            out_shape=jax.ShapeDtypeStruct(x.shape, x.dtype),
            scratch_shapes=[pltpu.VMEM((B, S, D), bf16), pltpu.VMEM((S, F), bf16), pltpu.VMEM((NC, 128), bf16), pltpu.VMEM((S, F), bf16),
                            pltpu.VMEM((1, S), bf16), pltpu.VMEM((NS, S, NT), bf16),
                            pltpu.VMEM((NG // 2 + 1, 8, 128), i32), pltpu.VMEM((NC + 3, S, NT), f32), pltpu.VMEM((len(allu), NP * KS + M, 8, 128), f32),
                            pltpu.VMEM((U + 1, KA // 2, NT), i32), [pltpu.VMEM((HE + 32, 128), f32)] * U, pltpu.VMEM((NS, 8, NT), i32), pltpu.VMEM((NS, NTV, 8, 128), f32), pltpu.VMEM((lead, 8, NT), f32),
                            pltpu.SemaphoreType.DMA((6,)), pltpu.SemaphoreType.DMA(())],
            compiler_params=pltpu.CompilerParams(vmem_limit_bytes=128 * 2**20, flags=flags, disable_bounds_checks=dbc),
        )(x, w1, b1.reshape(NC, 128), w2.T, b2.reshape(1, S))
    return fn


_fn = make(**dict(hpos=8))

@jax.jit
def pallas_standalone__mixer_token_mlp__sampling_kernel(x, w1, b1, w2, b2):
    return _fn(x, w1, b1, w2, b2)
```

```python
import numpy as np
import jax
import jax.numpy as jnp
from jax import lax
import jax.experimental.pallas as pl
import jax.experimental.pallas.tpu as pltpu

bf16, f32, i32 = jnp.bfloat16, jnp.float32, jnp.int32

_A = float(np.cbrt(0.044715 * np.sqrt(2 / np.pi)))
_K = float(np.sqrt(2 / np.pi)) / _A
_A_HI = float(np.float32(_A).astype(bf16))
_A_LO = _A - _A_HI
_EPS = 1e-5

LANES = 128
PANEL = 4 * LANES
KAUG = 32
ROW_STRIDE = 9
H_ROWS = 14 * 8 * ROW_STRIDE

UNROLL = 9
LEAD = 9
VPU_SLABS = 23
EARLY_TILES = 3
LN_PER_ITER = 4
STAGE_AT = 11


def _lanes(vs):
    return jnp.concatenate(list(vs), axis=-1)


def _rows(vs):
    return jnp.concatenate(list(vs), axis=0)


def _rows8(i):
    return pl.ds(8 * i if isinstance(i, int) else pl.multiple_of(8 * i, 8), 8)


def _pack(v):
    return pltpu.bitcast(v.astype(bf16), i32)


def _unpack(v):
    return pltpu.bitcast(v, bf16)


def _act(v):
    return v * jnp.tanh(v * (v * v + _K))


def _kernel(x_hbm, w1_hbm, b1_hbm, w2t_hbm, b2_hbm, o_hbm,
            x_v, w1_late_v, w1_early_v, b1_v, w2t_v, b2_v, o_v,
            w1t_s, w2_s, wvpu_s, h_s, hmxu_s, factor_s, carry_s, in_sems, out_sem, *hvpu_s):
    n_batch, n_tok, n_chan = x_v.shape
    n_tiles = b1_v.shape[0]
    n_slabs = 8 * n_tiles
    per_batch = n_chan // PANEL
    n_panels = n_batch * per_batch
    n_iter = (n_panels - 1) // UNROLL
    ln_ahead = max(min((1 + (i + 1) * UNROLL) // per_batch, n_batch - 1) + 1 - i * LN_PER_ITER
                   for i in range(n_iter))

    linear = n_slabs
    vpu_slabs = [int(round(6 + i * (n_slabs - 8) / (VPU_SLABS - 1))) for i in range(VPU_SLABS)]
    vpu_first = vpu_slabs[:2] + vpu_slabs[3:]

    def mxu_stream(on_vpu, linear_at):
        slabs, tile_ends = [], []
        for j in range(n_tiles):
            slabs += [linear] * (j == linear_at)
            slabs += [s for s in range(8 * j, 8 * j + 8) if s not in on_vpu]
            tile_ends.append(len(slabs))
        return slabs, tile_ends

    head = mxu_stream(vpu_first, 0)[0][:LEAD]

    def layernorm(b0, nb):
        x = _rows(x_v[b0 + b].astype(f32) for b in range(nb))
        xc = x - jnp.mean(x, axis=-1, keepdims=True)
        var = jnp.mean(xc * xc, axis=-1, keepdims=True)
        h = xc * (_A * lax.rsqrt(var + _EPS))
        for b in range(nb):
            for n in range(per_batch):
                h_s[_rows8((b0 + b) * per_batch + n), :] = _pack(
                    h[n_tok * b:n_tok * (b + 1), n * PANEL:(n + 1) * PANEL])

    def stage(panel, buf):
        packed = h_s[_rows8(panel), :]
        hmxu_s[buf, 0:8, :] = packed
        h = _unpack(packed).astype(f32)
        half = PANEL // 2
        b11, b12, b21, b22 = h[:8, :half], h[:8, half:], h[8:, :half], h[8:, half:]
        t1 = b12 - b11
        t2 = b22 - t1
        for p, v in enumerate([b11, b21, b22, t2 - b21, t1, t2, b22 - b12]):
            factor_s[buf, p] = v

    def spread(buf, p):
        for l in range(2):
            v = factor_s[buf, p, :, l * LANES:(l + 1) * LANES]
            for r in range(8):
                hvpu_s[buf][pl.ds((2 * p + l) * 8 * ROW_STRIDE + r, 8, stride=ROW_STRIDE), :] = v

    def build_vpu_weights():
        packed = [w1t_s[_rows8(slab), :] for slab in vpu_slabs]

        def column(i, s):
            v = _unpack(jnp.broadcast_to(packed[i][:, s:s + 1], (8, LANES))).astype(f32)
            return v[8:], v[:8]
        for i in range(VPU_SLABS):
            bias1, bias2 = column(i, n_tok)
            wvpu_s[i, 56 * 8:, :] = _rows([_A * bias1, _A * bias2 - _A * bias1])
        for s in range(8):
            for i in range(VPU_SLABS):
                (a11, a21), (a12, a22) = column(i, s), column(i, 8 + s)
                s1 = a21 + a22
                s2 = s1 - a11
                for p, v in enumerate([a11, a12, a12 - s2, a22, s1, s2, a11 - a21]):
                    wvpu_s[i, _rows8(8 * p + s), :] = v

    def matmul1_vpu(slab, buf):
        left = _lanes([wvpu_s[vpu_slabs.index(slab)]] * 2)
        prods = []
        for p in range(7):
            acc = left[448:456] if p == 0 else left[456:464] if p == 6 else None
            right = _lanes(_rows(hvpu_s[buf][pl.ds(((2 * p + l) * 8 + s) * ROW_STRIDE, 8), :]
                                 for s in range(8)) for l in range(2))
            terms = left[64 * p:64 * (p + 1)] * right
            for s in range(8):
                acc = terms[:8] if acc is None else acc + terms[8 * s:8 * s + 8]
            prods.append(acc)
        p1, p2, p3, p4, p5, p6, p7 = prods
        u2 = p1 + p6
        u3 = u2 + p7
        return _rows([_lanes([u3 - p4, u3 + p5]), _lanes([p1 + p2, (u2 + p5) + p3])])

    def matmul1_mxu(slabs, buf, a_rows=None):
        h = _unpack(hmxu_s[buf] if a_rows is None else _rows([hmxu_s[buf, 0:8, :], a_rows]))
        if linear in slabs:
            h = _rows([h, h])
        cuts = [i for i in range(len(slabs)) if i == 0 or slabs[i] != slabs[i - 1] + 1]
        w = _rows(w1t_s[8 * slabs[i]:8 * (slabs[e - 1] + 1), :]
                  for i, e in zip(cuts, cuts[1:] + [len(slabs)]))
        v = jnp.dot(_unpack(w)[:, :h.shape[0]], h, preferred_element_type=f32)
        return [v[16 * i:16 * i + 16] for i in range(len(slabs))]

    def write_back(panel):
        lane0 = panel % per_batch * PANEL
        if not isinstance(lane0, int):
            lane0 = pl.multiple_of(lane0, PANEL)
        pltpu.make_async_copy(
            o_v.at[panel], o_hbm.at[panel // per_batch, :, pl.ds(lane0, PANEL)], out_sem).start()

    def run_panels(panel0, plans, lead, side_work, zero=None):
        stream, ends = [], []
        for q, (_, on_vpu, linear_at) in enumerate(plans):
            slabs, tile_ends = mxu_stream(on_vpu, linear_at)
            ends += [len(stream) + e for e in tile_ends]
            stream += [(q, s) for s in slabs]
        stream += [(len(plans), s) for s in head]
        bufs = [plan[0] for plan in plans] + [0]
        pre = {} if zero is None else {(0, s): carry_s[i] for i, s in enumerate(head)}
        activated = list(pre)[:-1]
        pos = len(pre)
        sums = {}
        for t, tile_end in enumerate(ends):
            q, j = divmod(t, n_tiles)
            _, on_vpu, linear_at = plans[q]
            a_rows = side_work(q, j)
            stop = tile_end + lead if t + 1 < len(ends) else len(stream) - 1
            while pos < stop:
                chunk = [k for k in stream[pos:stop] if k[0] == stream[pos][0]]
                pre.update(zip(chunk, matmul1_mxu([s for _, s in chunk], bufs[chunk[0][0]], a_rows)))
                pos += len(chunk)
            keys = [(q, s) for s in range(8 * j + 7, 8 * j - 1, -1)]
            for _, s in keys:
                if s in on_vpu:
                    pre[q, s] = matmul1_vpu(s, bufs[q])
            if any(k in activated for k in keys):
                g = _rows(pre.pop(k) if k in activated else _act(pre.pop(k)) for k in keys)
            else:
                g = _act(_rows(pre.pop(k) for k in keys))
            tile = j
            if t - 2 in sums:
                w2_s[n_tiles] = pltpu.bitcast(sums.pop(t - 2), i32)
                tile = tile + zero
            y = lax.dot_general(_unpack(w2_s[tile, :8, :LANES]), g, (((1,), (0,)), ((), ())),
                                preferred_element_type=f32)
            total = y if j == 0 else total + y
            if j == linear_at:
                total = total + pre.pop((q, linear))
            if zero is not None and j % 4 == 3:
                sums[t] = total
            if j == n_tiles - 1:
                o_v[panel0 + q] = ((0.5 / _A) * total).astype(o_v.dtype)
        last, = matmul1_mxu(head[-1:], 0)
        for i, s in enumerate(head[:-1]):
            v = pre[len(plans), s]
            carry_s[i] = v if s == linear else _act(v)
        carry_s[LEAD - 1] = last

    n_late = w1_late_v.shape[1]
    rest = pl.ds(1, n_batch - 1)
    copies = [pltpu.make_async_copy(src, dst, in_sems.at[i]) for i, (src, dst) in enumerate([
        (x_hbm.at[0], x_v.at[0]), (w1_hbm.at[:, pl.ds(n_late, EARLY_TILES * LANES)], w1_early_v),
        (b1_hbm, b1_v), (w1_hbm.at[:, pl.ds(0, n_late)], w1_late_v), (w2t_hbm, w2t_v),
        (b2_hbm, b2_v), (x_hbm.at[rest], x_v.at[rest])])]
    for copy in copies[:6]:
        copy.start()

    row = lax.broadcasted_iota(i32, (16, LANES), 0)
    lane = lax.broadcasted_iota(i32, (16, LANES), 1)
    a_const = _pack(jnp.where(row == 0, _A_HI, jnp.where(row == 1, _A_LO, 0.0)))
    for buf in range(UNROLL):
        hmxu_s[buf, 8:16, :] = _lanes([a_const] * (PANEL // LANES))
        hvpu_s[buf][_rows8(H_ROWS // 8), :] = pltpu.bitcast(a_const, f32)

    for copy in copies[:3]:
        copy.wait()
    layernorm(0, 1)
    stage(0, 1)
    stage(1, 0)
    b1 = b1_v[...].astype(f32)
    w1_aug = {}
    for j in range(n_tiles):
        if j == EARLY_TILES:
            for copy in copies[3:6]:
                copy.wait()
            copies[6].start()
        c = n_tiles - 1 - j
        ref, col = (w1_early_v, c * LANES - n_late) if j < EARLY_TILES else (w1_late_v, c * LANES)
        bias = jnp.where(row < 2, jnp.broadcast_to(b1[c:c + 1, :], (16, LANES)), 0.0)
        w1_aug[c] = _rows([ref[:, col:col + LANES], bias.astype(bf16)])
        w1t = _rows([w1_aug[c], jnp.zeros((LANES - KAUG, LANES), bf16)]).T
        w1t_s[64 * j:64 * (j + 1), :] = _pack(_rows(w1t[k:k + 16] for k in range(112, -1, -16)))
    for c in range(n_tiles):
        w2_s[n_tiles - 1 - c, :8, :LANES] = _pack(w2t_v[:, c * LANES:(c + 1) * LANES])

    half = n_tiles // 2
    w12a, w12b = (
        lax.dot_general(w2t_v[:, c * LANES:(c + half) * LANES],
                        _lanes(w1_aug[c + k] for k in range(half)),
                        (((1,), (1,)), ((), ())), preferred_element_type=f32)
        for c in (0, half))
    w12 = _lanes([w12a + w12b, jnp.zeros((n_tok, LANES - KAUG), f32)])
    eye = (lax.broadcasted_iota(i32, (n_tok, n_tok), 0)
           == lax.broadcasted_iota(i32, (n_tok, n_tok), 1))
    b2 = jnp.sum(jnp.where(eye, jnp.broadcast_to(b2_v[...].astype(f32), (n_tok, n_tok)), 0.0),
                 axis=1, keepdims=True)
    w12 = w12 + jnp.where((lane == n_tok) | (lane == n_tok + 1), 2.0 * b2, 0.0)
    w12_hi = w12.astype(bf16).astype(f32)
    w1t_s[_rows8(linear), :] = _pack(w12_hi + pltpu.roll(w12 - w12_hi, KAUG, 1))

    def first_side_work(q, j):
        if j == 0:
            build_vpu_weights()
            for p in range(7):
                spread(0, p)
                spread(1, p)
        if j == n_tiles - 2:
            copies[6].wait()
            layernorm(1, ln_ahead - 1)

    run_panels(0, [(1, vpu_slabs[12:21], 20)], LEAD - 1, first_side_work)
    write_back(0)

    def iteration(it, parity):
        panel0 = 1 + it * UNROLL
        zero = parity * (1 - parity)

        rolled = pltpu.roll(wvpu_s[0, 0:8, :], 1, 1)

        def side_work(q, j):
            nxt = (q + 1) % UNROLL
            if j == (1 if q == 0 else 0):
                hvpu_s[q][_rows8(H_ROWS // 8 + 1 + zero), :] = rolled
            if q and j == 3:
                write_back(panel0 + q - 1)
            piece, off = divmod(j - STAGE_AT, 2)
            if off or not 0 <= piece < 7:
                return None
            if piece == 0:
                stage(jnp.minimum(panel0 + q + 1, n_panels - 1), nxt)
            spread(nxt, piece)
            a = hvpu_s[nxt][_rows8(H_ROWS // 8 + zero), :]
            return _lanes([pltpu.bitcast(a, i32)] * (PANEL // LANES))

        plans = [(q, vpu_slabs if q else vpu_first, 0) for q in range(UNROLL)]
        run_panels(panel0, plans, LEAD, side_work, zero)
        write_back(panel0 + UNROLL - 1)
        layernorm(jnp.minimum(ln_ahead + it * LN_PER_ITER, n_batch - LN_PER_ITER), LN_PER_ITER)
        return 1 - parity

    lax.fori_loop(0, n_iter, iteration, 0)
    pltpu.make_async_copy(o_hbm, o_hbm, out_sem).wait()


@jax.jit
def pallas_standalone__mixer_token_mlp__sampling_kernel(
    x: jax.Array,
    w1: jax.Array,
    b1: jax.Array,
    w2: jax.Array,
    b2: jax.Array,
):
    n_batch, n_tok, n_chan = x.shape
    n_hidden = w1.shape[1]
    n_tiles = n_hidden // LANES
    n_panels = n_batch * n_chan // PANEL
    assert n_tok == 16 and n_chan == 2 * PANEL and n_hidden == 28 * LANES
    assert (n_panels - 1) % UNROLL == 0
    hbm = pl.BlockSpec(memory_space=pltpu.HBM)
    return pl.pallas_call(
        _kernel,
        in_specs=[hbm] * 5,
        out_specs=hbm,
        out_shape=jax.ShapeDtypeStruct(x.shape, x.dtype),
        scratch_shapes=[
            pltpu.VMEM(x.shape, x.dtype),
            pltpu.VMEM((n_tok, n_hidden - EARLY_TILES * LANES), w1.dtype),
            pltpu.VMEM((n_tok, EARLY_TILES * LANES), w1.dtype),
            pltpu.VMEM((n_tiles, LANES), b1.dtype),
            pltpu.VMEM((n_tok, n_hidden), w2.dtype),
            pltpu.VMEM((1, n_tok), b2.dtype),
            pltpu.VMEM((n_panels, n_tok, PANEL), x.dtype),
            pltpu.VMEM(((8 * n_tiles + 1) * 8, LANES), i32),
            pltpu.VMEM((n_tiles + 1, n_tok, PANEL), i32),
            pltpu.VMEM((VPU_SLABS, 58 * 8, LANES), f32),
            pltpu.VMEM((n_panels * 8, PANEL), i32),
            pltpu.VMEM((UNROLL, KAUG // 2, PANEL), i32),
            pltpu.VMEM((UNROLL, 7, 8, PANEL // 2), f32),
            pltpu.VMEM((LEAD, 16, PANEL), f32),
            pltpu.SemaphoreType.DMA((7,)),
            pltpu.SemaphoreType.DMA(()),
        ] + [pltpu.VMEM((H_ROWS + 16, LANES), f32)] * UNROLL,
        compiler_params=pltpu.CompilerParams(
            vmem_limit_bytes=128 * 2**20, disable_bounds_checks=True),
    )(x, w1, b1.reshape(n_tiles, LANES), w2.T, b2.reshape(1, n_tok))
```

```python
import numpy as np
import jax
import jax.numpy as jnp
from jax import lax
import jax.experimental.pallas as pl
import jax.experimental.pallas.tpu as pltpu

bf16, f32, i32 = jnp.bfloat16, jnp.float32, jnp.int32

_A = float(np.cbrt(0.044715 * np.sqrt(2 / np.pi)))
_K = float(np.sqrt(2 / np.pi)) / _A
_A_HI = float(np.float32(_A).astype(bf16))
_A_LO = _A - _A_HI
_EPS = 1e-5

LANES = 128
PANEL = 4 * LANES
KAUG = 32
ROW_STRIDE = 9
H_ROWS = 14 * 8 * ROW_STRIDE

UNROLL = 9
LEAD = 9
VPU_SLABS = 23
EARLY_TILES = 3
LN_PER_ITER = 4
STAGE_AT = 13


def _lanes(vs):
    return jnp.concatenate(list(vs), axis=-1)


def _rows(vs):
    return jnp.concatenate(list(vs), axis=0)


def _rows8(i):
    return pl.ds(8 * i if isinstance(i, int) else pl.multiple_of(8 * i, 8), 8)


def _pack(v):
    return pltpu.bitcast(v.astype(bf16), i32)


def _unpack(v):
    return pltpu.bitcast(v, bf16)


def _act(v):
    return v * jnp.tanh(v * (v * v + _K))


def _kernel(x_hbm, w1_hbm, b1_hbm, w2t_hbm, b2_hbm, o_hbm,
            x_v, w1_late_v, w1_early_v, b1_v, w2t_v, b2_v, o_v,
            w1t_s, w2_s, wvpu_s, h_s, hmxu_s, factor_s, carry_s, in_sems, out_sem, *hvpu_s):
    n_batch, n_tok, n_chan = x_v.shape
    n_tiles = b1_v.shape[0]
    n_slabs = 8 * n_tiles
    per_batch = n_chan // PANEL
    n_panels = n_batch * per_batch
    n_iter = (n_panels - 1) // UNROLL
    ln_ahead = max(min((1 + (i + 1) * UNROLL) // per_batch, n_batch - 1) + 1 - i * LN_PER_ITER
                   for i in range(n_iter))

    linear = n_slabs
    vpu_slabs = [int(round(6 + i * (n_slabs - 8) / (VPU_SLABS - 1))) for i in range(VPU_SLABS)]
    vpu_first = vpu_slabs[:2] + vpu_slabs[3:]

    def mxu_stream(on_vpu, linear_at):
        slabs, tile_ends = [], []
        for j in range(n_tiles):
            slabs += [linear] * (j == linear_at)
            slabs += [s for s in range(8 * j, 8 * j + 8) if s not in on_vpu]
            tile_ends.append(len(slabs))
        return slabs, tile_ends

    head = mxu_stream(vpu_first, 0)[0][:LEAD]

    def layernorm(b0, nb):
        x = _rows(x_v[b0 + b].astype(f32) for b in range(nb))
        xc = x - jnp.mean(x, axis=-1, keepdims=True)
        var = jnp.mean(xc * xc, axis=-1, keepdims=True)
        h = xc * (_A * lax.rsqrt(var + _EPS))
        for b in range(nb):
            for n in range(per_batch):
                h_s[_rows8((b0 + b) * per_batch + n), :] = _pack(
                    h[n_tok * b:n_tok * (b + 1), n * PANEL:(n + 1) * PANEL])

    def stage(panel, buf):
        packed = h_s[_rows8(panel), :]
        hmxu_s[buf, 0:8, :] = packed
        h = _unpack(packed).astype(f32)
        half = PANEL // 2
        b11, b12, b21, b22 = h[:8, :half], h[:8, half:], h[8:, :half], h[8:, half:]
        t1 = b12 - b11
        t2 = b22 - t1
        for p, v in enumerate([b11, b21, b22, t2 - b21, t1, t2, b22 - b12]):
            factor_s[buf, p] = v

    def spread(buf, p):
        for l in range(2):
            v = factor_s[buf, p, :, l * LANES:(l + 1) * LANES]
            for r in range(8):
                hvpu_s[buf][pl.ds((2 * p + l) * 8 * ROW_STRIDE + r, 8, stride=ROW_STRIDE), :] = v

    def load_spread(buf):
        return [_lanes(_rows(hvpu_s[buf][pl.ds(((2 * p + l) * 8 + s) * ROW_STRIDE, 8), :]
                             for s in range(8)) for l in range(2)) for p in range(7)]

    def build_vpu_weights():
        packed = [w1t_s[_rows8(slab), :] for slab in vpu_slabs]

        def column(i, s):
            v = _unpack(jnp.broadcast_to(packed[i][:, s:s + 1], (8, LANES))).astype(f32)
            return v[8:], v[:8]
        for i in range(VPU_SLABS):
            bias1, bias2 = column(i, n_tok)
            wvpu_s[i, 56 * 8:, :] = _rows([_A * bias1, _A * bias2 - _A * bias1])
        for s in range(8):
            for i in range(VPU_SLABS):
                (a11, a21), (a12, a22) = column(i, s), column(i, 8 + s)
                s1 = a21 + a22
                s2 = s1 - a11
                for p, v in enumerate([a11, a12, a12 - s2, a22, s1, s2, a11 - a21]):
                    wvpu_s[i, _rows8(8 * p + s), :] = v

    def matmul1_vpu(slab, right):
        left = _lanes([wvpu_s[vpu_slabs.index(slab)]] * 2)
        prods = []
        for p in range(7):
            acc = left[448:456] if p == 0 else left[456:464] if p == 6 else None
            terms = left[64 * p:64 * (p + 1)] * right[p]
            for s in range(8):
                acc = terms[:8] if acc is None else acc + terms[8 * s:8 * s + 8]
            prods.append(acc)
        p1, p2, p3, p4, p5, p6, p7 = prods
        u2 = p1 + p6
        u3 = u2 + p7
        return _rows([_lanes([u3 - p4, u3 + p5]), _lanes([p1 + p2, (u2 + p5) + p3])])

    def matmul1_mxu(slabs, buf, a_rows=None):
        h = _unpack(hmxu_s[buf] if a_rows is None else _rows([hmxu_s[buf, 0:8, :], a_rows]))
        if linear in slabs:
            h = _rows([h, h])
        cuts = [i for i in range(len(slabs)) if i == 0 or slabs[i] != slabs[i - 1] + 1]
        w = _rows(w1t_s[8 * slabs[i]:8 * (slabs[e - 1] + 1), :]
                  for i, e in zip(cuts, cuts[1:] + [len(slabs)]))
        v = jnp.dot(_unpack(w)[:, :h.shape[0]], h, preferred_element_type=f32)
        return [v[16 * i:16 * i + 16] for i in range(len(slabs))]

    def write_back(panel):
        lane0 = panel % per_batch * PANEL
        if not isinstance(lane0, int):
            lane0 = pl.multiple_of(lane0, PANEL)
        pltpu.make_async_copy(
            o_v.at[panel], o_hbm.at[panel // per_batch, :, pl.ds(lane0, PANEL)], out_sem).start()

    def run_panels(panel0, plans, lead, side_work, zero=None):
        stream, ends = [], []
        for q, (_, on_vpu, linear_at) in enumerate(plans):
            slabs, tile_ends = mxu_stream(on_vpu, linear_at)
            ends += [len(stream) + e for e in tile_ends]
            stream += [(q, s) for s in slabs]
        stream += [(len(plans), s) for s in head]
        bufs = [plan[0] for plan in plans] + [0]
        pre = {} if zero is None else {(0, s): carry_s[i] for i, s in enumerate(head)}
        activated = list(pre)[:-1]
        pos = len(pre)
        sums = {}
        for t, tile_end in enumerate(ends):
            q, j = divmod(t, n_tiles)
            _, on_vpu, linear_at = plans[q]
            a_rows = side_work(q, j)
            stop = tile_end + lead if t + 1 < len(ends) else len(stream) - 1
            while pos < stop:
                chunk = [k for k in stream[pos:stop] if k[0] == stream[pos][0]]
                pre.update(zip(chunk, matmul1_mxu([s for _, s in chunk], bufs[chunk[0][0]], a_rows)))
                pos += len(chunk)
            keys = [(q, s) for s in range(8 * j + 7, 8 * j - 1, -1)]
            if j == 0 or (zero is not None and q == 0 and j % 2):
                right = load_spread(bufs[q])
            for _, s in keys:
                if s in on_vpu:
                    pre[q, s] = matmul1_vpu(s, right)
            if any(k in activated for k in keys):
                g = _rows(pre.pop(k) if k in activated else _act(pre.pop(k)) for k in keys)
            else:
                g = _act(_rows(pre.pop(k) for k in keys))
            tile = j
            if t - 2 in sums:
                w2_s[n_tiles] = pltpu.bitcast(sums.pop(t - 2), i32)
                tile = tile + zero
            y = lax.dot_general(_unpack(w2_s[tile, :8, :LANES]), g, (((1,), (0,)), ((), ())),
                                preferred_element_type=f32)
            total = y if j == 0 else total + y
            if j == linear_at:
                total = total + pre.pop((q, linear))
            if zero is not None and j % 4 == 3:
                sums[t] = total
            if j == n_tiles - 1:
                o_v[panel0 + q] = ((0.5 / _A) * total).astype(o_v.dtype)
        last, = matmul1_mxu(head[-1:], 0)
        for i, s in enumerate(head[:-1]):
            v = pre[len(plans), s]
            carry_s[i] = v if s == linear else _act(v)
        carry_s[LEAD - 1] = last

    n_late = w1_late_v.shape[1]
    rest = pl.ds(1, n_batch - 1)
    copies = [pltpu.make_async_copy(src, dst, in_sems.at[i]) for i, (src, dst) in enumerate([
        (x_hbm.at[0], x_v.at[0]), (w1_hbm.at[:, pl.ds(n_late, EARLY_TILES * LANES)], w1_early_v),
        (b1_hbm, b1_v), (w1_hbm.at[:, pl.ds(0, n_late)], w1_late_v), (w2t_hbm, w2t_v),
        (b2_hbm, b2_v), (x_hbm.at[rest], x_v.at[rest])])]
    for copy in copies[:6]:
        copy.start()

    row = lax.broadcasted_iota(i32, (16, LANES), 0)
    lane = lax.broadcasted_iota(i32, (16, LANES), 1)
    a_const = _pack(jnp.where(row == 0, _A_HI, jnp.where(row == 1, _A_LO, 0.0)))
    for buf in range(UNROLL):
        hmxu_s[buf, 8:16, :] = _lanes([a_const] * (PANEL // LANES))
        hvpu_s[buf][_rows8(H_ROWS // 8), :] = pltpu.bitcast(a_const, f32)

    for copy in copies[:3]:
        copy.wait()
    layernorm(0, 1)
    stage(0, 1)
    stage(1, 0)
    b1 = b1_v[...].astype(f32)
    w1_aug = {}
    for j in range(n_tiles):
        if j == EARLY_TILES:
            for copy in copies[3:6]:
                copy.wait()
            copies[6].start()
        c = n_tiles - 1 - j
        ref, col = (w1_early_v, c * LANES - n_late) if j < EARLY_TILES else (w1_late_v, c * LANES)
        bias = jnp.where(row < 2, jnp.broadcast_to(b1[c:c + 1, :], (16, LANES)), 0.0)
        w1_aug[c] = _rows([ref[:, col:col + LANES], bias.astype(bf16)])
        w1t = _rows([w1_aug[c], jnp.zeros((LANES - KAUG, LANES), bf16)]).T
        w1t_s[64 * j:64 * (j + 1), :] = _pack(_rows(w1t[k:k + 16] for k in range(112, -1, -16)))
    for c in range(n_tiles):
        w2_s[n_tiles - 1 - c, :8, :LANES] = _pack(w2t_v[:, c * LANES:(c + 1) * LANES])

    half = n_tiles // 2
    w12a, w12b = (
        lax.dot_general(w2t_v[:, c * LANES:(c + half) * LANES],
                        _lanes(w1_aug[c + k] for k in range(half)),
                        (((1,), (1,)), ((), ())), preferred_element_type=f32)
        for c in (0, half))
    w12 = _lanes([w12a + w12b, jnp.zeros((n_tok, LANES - KAUG), f32)])
    eye = (lax.broadcasted_iota(i32, (n_tok, n_tok), 0)
           == lax.broadcasted_iota(i32, (n_tok, n_tok), 1))
    b2 = jnp.sum(jnp.where(eye, jnp.broadcast_to(b2_v[...].astype(f32), (n_tok, n_tok)), 0.0),
                 axis=1, keepdims=True)
    w12 = w12 + jnp.where((lane == n_tok) | (lane == n_tok + 1), 2.0 * b2, 0.0)
    w12_hi = w12.astype(bf16).astype(f32)
    w1t_s[_rows8(linear), :] = _pack(w12_hi + pltpu.roll(w12 - w12_hi, KAUG, 1))

    def first_side_work(q, j):
        if j == 0:
            build_vpu_weights()
            for p in range(7):
                spread(0, p)
                spread(1, p)
        if j == n_tiles - 2:
            copies[6].wait()
            layernorm(1, ln_ahead - 1)

    run_panels(0, [(1, vpu_slabs[12:21], 20)], LEAD - 1, first_side_work)
    write_back(0)

    def iteration(it, parity):
        panel0 = 1 + it * UNROLL
        zero = parity * (1 - parity)

        rolled = pltpu.roll(wvpu_s[0, 0:8, :], 1, 1)

        def side_work(q, j):
            nxt = (q + 1) % UNROLL
            if j == (1 if q == 0 else 0):
                hvpu_s[q][_rows8(H_ROWS // 8 + 1 + zero), :] = rolled
            if q and j == 3:
                write_back(panel0 + q - 1)
            piece, off = divmod(j - STAGE_AT, 2)
            if off or not 0 <= piece < 7:
                return None
            if piece == 0:
                stage(jnp.minimum(panel0 + q + 1, n_panels - 1), nxt)
            spread(nxt, piece)
            a = hvpu_s[nxt][_rows8(H_ROWS // 8 + zero), :]
            return _lanes([pltpu.bitcast(a, i32)] * (PANEL // LANES))

        plans = [(q, vpu_slabs if q else vpu_first, 0) for q in range(UNROLL)]
        run_panels(panel0, plans, LEAD, side_work, zero)
        write_back(panel0 + UNROLL - 1)
        layernorm(jnp.minimum(ln_ahead + it * LN_PER_ITER, n_batch - LN_PER_ITER), LN_PER_ITER)
        return 1 - parity

    lax.fori_loop(0, n_iter, iteration, 0)
    pltpu.make_async_copy(o_hbm, o_hbm, out_sem).wait()


@jax.jit
def pallas_standalone__mixer_token_mlp__sampling_kernel(
    x: jax.Array,
    w1: jax.Array,
    b1: jax.Array,
    w2: jax.Array,
    b2: jax.Array,
):
    n_batch, n_tok, n_chan = x.shape
    n_hidden = w1.shape[1]
    n_tiles = n_hidden // LANES
    n_panels = n_batch * n_chan // PANEL
    assert n_tok == 16 and n_chan == 2 * PANEL and n_hidden == 28 * LANES
    assert (n_panels - 1) % UNROLL == 0
    hbm = pl.BlockSpec(memory_space=pltpu.HBM)
    return pl.pallas_call(
        _kernel,
        in_specs=[hbm] * 5,
        out_specs=hbm,
        out_shape=jax.ShapeDtypeStruct(x.shape, x.dtype),
        scratch_shapes=[
            pltpu.VMEM(x.shape, x.dtype),
            pltpu.VMEM((n_tok, n_hidden - EARLY_TILES * LANES), w1.dtype),
            pltpu.VMEM((n_tok, EARLY_TILES * LANES), w1.dtype),
            pltpu.VMEM((n_tiles, LANES), b1.dtype),
            pltpu.VMEM((n_tok, n_hidden), w2.dtype),
            pltpu.VMEM((1, n_tok), b2.dtype),
            pltpu.VMEM((n_panels, n_tok, PANEL), x.dtype),
            pltpu.VMEM(((8 * n_tiles + 1) * 8, LANES), i32),
            pltpu.VMEM((n_tiles + 1, n_tok, PANEL), i32),
            pltpu.VMEM((VPU_SLABS, 58 * 8, LANES), f32),
            pltpu.VMEM((n_panels * 8, PANEL), i32),
            pltpu.VMEM((UNROLL, KAUG // 2, PANEL), i32),
            pltpu.VMEM((UNROLL, 7, 8, PANEL // 2), f32),
            pltpu.VMEM((LEAD, 16, PANEL), f32),
            pltpu.SemaphoreType.DMA((7,)),
            pltpu.SemaphoreType.DMA(()),
        ] + [pltpu.VMEM((H_ROWS + 16, LANES), f32)] * UNROLL,
        compiler_params=pltpu.CompilerParams(
            vmem_limit_bytes=128 * 2**20, disable_bounds_checks=True),
    )(x, w1, b1.reshape(n_tiles, LANES), w2.T, b2.reshape(1, n_tok))
```
